```python
import jax
import jax.numpy as jnp

def _softmax(x, axis=-1):
    return jax.nn.softmax(x, axis=axis)

def _gelu(x):
    return jax.nn.gelu(x, approximate=True)

def _silu(x):
    return jax.nn.silu(x)

def _sigmoid(x):
    return jax.nn.sigmoid(x)

def _layernorm(x, axis=-1, eps=1e-05):
    m = jnp.mean(x, axis=axis, keepdims=True)
    v = jnp.var(x, axis=axis, keepdims=True)
    return (x - m) / jnp.sqrt(v + eps)

def _scatter_add(tgt, idx, src, axis=0):
    return tgt.at[idx].add(src)

def _segment_sum(src, seg, n):
    return jax.ops.segment_sum(src, seg, n)

class _Rng:

    def __init__(self, key):
        self._k = key

    def _next(self):
        self._k, sub = jax.random.split(self._k)
        return sub

    def normal(self, shape):
        return jax.random.normal(self._next(), shape, dtype=jnp.bfloat16)

    def randint(self, lo, hi, shape):
        return jax.random.randint(self._next(), shape, lo, hi, dtype=jnp.int32)

    def uniform(self, shape, lo=0.0, hi=1.0):
        return jax.random.uniform(self._next(), shape, jnp.bfloat16, lo, hi)

    def permutation(self, n):
        return jax.random.permutation(self._next(), n)
kernel_name = 'recurrent_scan__memory_aug_recurrent_mem_tr__glu_gated_glu__prompt'

def setup_inputs():
    _rng = _Rng(jax.random.key(int.from_bytes(__import__("os").urandom(4), "little")))
    _w = lambda a: (lambda t: t.astype(jnp.bfloat16) if jnp.issubdtype(t.dtype, jnp.floating) else t)(jnp.asarray(a))

    def _A_setup():
        B, S, Dm = (1, 2048, 1024)
        H, Dh = (32, 128)
        M, seg = (8, 32)
        seg = min(seg, S)
        S = S // seg * seg
        return {'x': _w((lambda *s: _rng.normal(s) * 0.05)(B, S, Dm)), 'mem0': _w((lambda *s: _rng.normal(s) * 0.05)(B, M, Dm)), 'Wq': _w((lambda *s: _rng.normal(s) * 0.05)(Dm, H, Dh) * Dm ** (-0.5)), 'Wk': _w((lambda *s: _rng.normal(s) * 0.05)(Dm, H, Dh) * Dm ** (-0.5)), 'Wv': _w((lambda *s: _rng.normal(s) * 0.05)(Dm, H, Dh) * Dm ** (-0.5)), 'Wo': _w((lambda *s: _rng.normal(s) * 0.05)(H, Dh, Dm) * (H * Dh) ** (-0.5)), 'seg_len': seg}
    _A_in = _A_setup()

    def _B_setup():
        B, S, D, F = (1, 2048, 1024, 3584)
        return {'x': _w((lambda *s: _rng.normal(s) * 0.05)(B, S, D)), 'w_gate': _w((lambda *s: _rng.normal(s) * 0.05)(D, F)), 'w_up': _w((lambda *s: _rng.normal(s) * 0.05)(D, F)), 'w_down': _w((lambda *s: _rng.normal(s) * 0.05)(F, D))}
    _B_in = _B_setup()
    return {'A_x': _A_in['x'], 'A_mem0': _A_in['mem0'], 'A_Wq': _A_in['Wq'], 'A_Wk': _A_in['Wk'], 'A_Wv': _A_in['Wv'], 'A_Wo': _A_in['Wo'], 'A_seg_len': _A_in['seg_len'], 'B_x': _B_in['x'], 'B_w_gate': _B_in['w_gate'], 'B_w_up': _B_in['w_up'], 'B_w_down': _B_in['w_down']}

def reference(A_x, A_mem0, A_Wq, A_Wk, A_Wv, A_Wo, A_seg_len, B_x, B_w_gate, B_w_up, B_w_down):

    def _A_ref(x, mem0, Wq, Wk, Wv, Wo, seg_len):
        B, S, Dm = x.shape
        H, Dh = (Wq.shape[1], Wq.shape[2])
        M = mem0.shape[1]
        scale = Dh ** (-0.5)
        n_seg = S // seg_len
        L = M + seg_len
        idx = jnp.arange(L)
        mask = (idx[:, None] < M) | (idx[:, None] >= idx[None, :])
        mem = mem0
        outs = []
        for s in range(n_seg):
            xs = x[:, s * seg_len:(s + 1) * seg_len, :].copy()
            h = jnp.concatenate([mem, xs], axis=1)
            q = jnp.einsum('btd,dhe->bhte', h, Wq)
            k = jnp.einsum('btd,dhe->bhte', h, Wk)
            v = jnp.einsum('btd,dhe->bhte', h, Wv)
            scores = jnp.einsum('bhqe,bhke->bhqk', q, k) * scale
            scores = jnp.where(mask[None, None], scores, -1000000000.0)
            p = _softmax(scores, axis=-1)
            o = jnp.einsum('bhqk,bhke->bhqe', p, v)
            o = jnp.einsum('bhte,hed->btd', o, Wo)
            mem = o[:, :M, :].copy()
            outs.append(o[:, M:, :])
        return jnp.concatenate(outs, axis=1)

    def _B_ref(x, w_gate, w_up, w_down):
        g = jnp.einsum('bsd,df->bsf', x, w_gate)
        u = jnp.einsum('bsd,df->bsf', x, w_up)
        h = _sigmoid(g) * u
        return jnp.einsum('bsf,fd->bsd', h, w_down)
    x = A_x
    xn = _layernorm(x, axis=-1)
    s = _A_ref(xn, A_mem0, A_Wq, A_Wk, A_Wv, A_Wo, A_seg_len)
    g = _silu(_B_ref(xn, B_w_gate, B_w_up, B_w_down))
    return x + s * g
```

```python
import functools

import jax
import jax.numpy as jnp
from jax import lax
import jax.experimental.pallas as pl
import jax.experimental.pallas.tpu as pltpu

_F32 = jnp.float32
_BF16 = jnp.bfloat16
_U32 = jnp.uint32

_TB = 256
_FC = 512
_HG = 4
_DC = 64


def _dot(a, b):
    return jnp.dot(a, b, preferred_element_type=_F32)


def _unpack_w(w32):
    return pltpu.bitcast(w32, _BF16)


def _kernel(x_hbm, mem0_ref, wq_hbm, wk_hbm, wv_hbm, wo_hbm, wg_hbm, wu_hbm, wd_hbm,
            out_hbm,
            x_v, xn32, xn16, acc, out_v, wqkv, wo_p, qstage, ostage, wg_b, wu_b, wd_b,
            sem_x, sem_g, sem_r, sem_o,
            *, S, D, H, Dh, M, seg, F):
    n_seg = S // seg
    n_tb = S // _TB
    n_fc = F // _FC
    n_dc = D // _DC
    n_it = n_tb * n_fc
    n_qkv_units = 3 * n_dc
    n_wo_units = n_it - n_qkv_units
    wo_rows = (H * Dh) // n_wo_units
    scale = Dh ** -0.5

    def glu_copies(fc, slot):
        return (
            pltpu.make_async_copy(wg_hbm.at[:, pl.ds(fc * _FC, _FC)], wg_b.at[slot], sem_g.at[0, slot]),
            pltpu.make_async_copy(wu_hbm.at[:, pl.ds(fc * _FC, _FC)], wu_b.at[slot], sem_g.at[1, slot]),
            pltpu.make_async_copy(wd_hbm.at[pl.ds(fc * _FC, _FC), :], wd_b.at[slot], sem_g.at[2, slot]),
        )

    def qkv_copy(w_hbm, dc, slot):
        return pltpu.make_async_copy(
            w_hbm.bitcast(_U32).at[pl.ds(dc * (_DC * H // 2), _DC * H // 2)],
            qstage.at[slot], sem_r.at[slot])

    def wo_copy(u, slot):
        return pltpu.make_async_copy(
            wo_hbm.at[pl.ds(u * wo_rows, wo_rows), :], ostage.at[slot], sem_r.at[slot])

    x_copy = pltpu.make_async_copy(x_hbm, x_v, sem_x.at[0])
    x_copy.start()
    for c in glu_copies(0, 0):
        c.start()
    qkv_copy(wq_hbm, 0, 0).start()
    x_copy.wait()

    def ln_body(i, carry):
        rows = pl.ds(pl.multiple_of(i * _TB, _TB), _TB)
        xf = x_v[rows, :].astype(_F32)
        mu = jnp.mean(xf, axis=-1, keepdims=True)
        xc = xf - mu
        var = jnp.mean(xc * xc, axis=-1, keepdims=True)
        xn = xc * lax.rsqrt(var + 1e-5)
        xb = xn.astype(_BF16)
        xn16[rows, :] = xb
        xn32[rows, :] = xb.astype(_F32)
        return carry

    lax.fori_loop(0, n_tb, ln_body, 0)

    def glu_unit(it):
        fc = it // n_tb
        tb = it % n_tb
        slot = fc % 2
        rows = pl.ds(pl.multiple_of(tb * _TB, _TB), _TB)
        xb = xn16[rows, :]
        g = _dot(xb, wg_b[slot])
        u = _dot(xb, wu_b[slot])
        h = (jax.nn.sigmoid(g) * u).astype(_BF16)
        y = _dot(h, wd_b[slot])
        prev = acc[rows, :]
        acc[rows, :] = jnp.where(fc == 0, y, prev + y)

    def glu_dma(it):
        fc = it // n_tb
        tb = it % n_tb
        slot = fc % 2

        @pl.when(tb == 0)
        def _():
            @pl.when(fc + 1 < n_fc)
            def _():
                for c in glu_copies(fc + 1, 1 - slot):
                    c.start()
            for c in glu_copies(fc, slot):
                c.wait()

    def qkv_body(it, carry):
        glu_dma(it)
        m = it // n_dc
        dc = it % n_dc
        slot = it % 2
        nxt = it + 1
        nm = nxt // n_dc
        ndc = nxt % n_dc
        for mm, w_hbm in enumerate((wq_hbm, wk_hbm, wv_hbm)):
            @pl.when(nm == mm)
            def _():
                qkv_copy(w_hbm, ndc, 1 - slot).start()

        @pl.when(nm == 3)
        def _():
            wo_copy(0, 1 - slot).start()
        qkv_copy(wq_hbm, dc, slot).wait()

        glu_unit(it)

        half = _DC // 2
        drows = pl.ds(pl.multiple_of(dc * half, half), half)
        for j in range(H // 2):
            a = qstage[slot, pl.ds(j, half, stride=H), :]
            b = qstage[slot, pl.ds(H // 2 + j, half, stride=H), :]
            lo = (a & jnp.uint32(0xFFFF)) | (b << 16)
            hi = (a >> 16) | (b & jnp.uint32(0xFFFF0000))
            wqkv[2 * j, m, drows, :] = lo
            wqkv[2 * j + 1, m, drows, :] = hi
        return carry

    lax.fori_loop(0, n_qkv_units, qkv_body, 0)

    def wo_body(u, carry):
        it = n_qkv_units + u
        glu_dma(it)
        slot = it % 2

        @pl.when(u + 1 < n_wo_units)
        def _():
            wo_copy(u + 1, 1 - slot).start()
        wo_copy(u, slot).wait()

        glu_unit(it)

        wo_p[pl.ds(pl.multiple_of(u * (wo_rows // 2), wo_rows // 2), wo_rows // 2), :] = (
            pltpu.bitcast(ostage[slot], _U32))
        return carry

    lax.fori_loop(0, n_wo_units, wo_body, 0)

    L = M + seg
    Lp = 48
    row_i = lax.broadcasted_iota(jnp.int32, (Lp, Lp), 0)
    col_i = lax.broadcasted_iota(jnp.int32, (Lp, Lp), 1)
    mask = ((row_i < M) | (row_i >= col_i)) & (col_i < L)

    def seg_body(s, mem):
        r0 = pl.multiple_of(s * seg, seg)
        xs = xn32[pl.ds(r0, seg), :]
        hs = jnp.concatenate([mem, xs, jnp.zeros((Lp - L, D), _F32)], axis=0).astype(_BF16)
        G = _HG
        n_g = H // G
        qkv, probs, outs = {}, {}, {}
        o_acc = None
        for i in range(n_g + 3):
            if i < n_g:
                qkv[i] = [
                    tuple(_dot(hs, _unpack_w(wqkv[h, t])).astype(_BF16) for t in range(3))
                    for h in range(i * G, (i + 1) * G)]
            g1 = i - 1
            if 0 <= g1 < n_g:
                ps = []
                for (q, k, v) in qkv[g1]:
                    sc = lax.dot_general(q, k, (((1,), (1,)), ((), ())),
                                         preferred_element_type=_F32) * scale
                    sc = jnp.where(mask, sc, -1e9)
                    mx = jnp.max(sc, axis=-1, keepdims=True)
                    e = jnp.exp(sc - mx)
                    ps.append((e / jnp.sum(e, axis=-1, keepdims=True)).astype(_BF16))
                probs[g1] = ps
            g2 = i - 2
            if 0 <= g2 < n_g:
                outs[g2] = jnp.concatenate(
                    [_dot(p, v).astype(_BF16) for p, (_, _, v) in zip(probs[g2], qkv[g2])], axis=1)
            g3 = i - 3
            if 0 <= g3 < n_g:
                r = G * Dh // 2
                y = _dot(outs[g3], _unpack_w(wo_p[g3 * r:(g3 + 1) * r, :]))
                o_acc = y if o_acc is None else o_acc + y
        rows = pl.ds(r0, seg)
        g = acc[rows, :]
        g = g * jax.nn.sigmoid(g)
        out_v[rows, :] = (x_v[rows, :].astype(_F32) + o_acc[M:L, :] * g).astype(out_v.dtype)
        pltpu.make_async_copy(out_v.at[rows, :], out_hbm.at[rows, :], sem_o.at[0]).start()
        return o_acc[:M, :].astype(_BF16).astype(_F32)

    lax.fori_loop(0, n_seg, seg_body, mem0_ref[...].astype(_F32))
    pltpu.make_async_copy(out_v, out_hbm, sem_o.at[0]).wait()


@functools.partial(jax.jit, static_argnames=("A_seg_len",))
def pallas_recurrent_scan__memory_aug_recurrent_mem_tr__glu_gated_glu__prompt_kernel(
    A_x, A_mem0, A_Wq, A_Wk, A_Wv, A_Wo, A_seg_len, B_x, B_w_gate, B_w_up, B_w_down,
):
    del B_x
    B, S, D = A_x.shape
    _, H, Dh = A_Wq.shape
    M = A_mem0.shape[1]
    F = B_w_gate.shape[1]
    seg = int(A_seg_len)
    assert B == 1 and Dh == 128 and M == 8 and seg == 32 and D == 1024 and H == 32
    assert S % _TB == 0 and F % _FC == 0

    n_it = (S // _TB) * (F // _FC)
    n_wo_units = n_it - 3 * (D // _DC)
    wo_rows = (H * Dh) // n_wo_units

    hbm = pl.BlockSpec(memory_space=pl.ANY)
    kern = functools.partial(_kernel, S=S, D=D, H=H, Dh=Dh, M=M, seg=seg, F=F)
    out = pl.pallas_call(
        kern,
        out_shape=jax.ShapeDtypeStruct((S, D), A_x.dtype),
        in_specs=[hbm, pl.BlockSpec(memory_space=pltpu.VMEM), hbm, hbm, hbm, hbm, hbm, hbm, hbm],
        out_specs=hbm,
        scratch_shapes=[
            pltpu.VMEM((S, D), _BF16),
            pltpu.VMEM((S, D), _F32),
            pltpu.VMEM((S, D), _BF16),
            pltpu.VMEM((S, D), _F32),
            pltpu.VMEM((S, D), A_x.dtype),
            pltpu.VMEM((H, 3, D // 2, Dh), _U32),
            pltpu.VMEM((H * Dh // 2, D), _U32),
            pltpu.VMEM((2, _DC * H // 2, Dh), _U32),
            pltpu.VMEM((2, wo_rows, D), _BF16),
            pltpu.VMEM((2, D, _FC), _BF16),
            pltpu.VMEM((2, D, _FC), _BF16),
            pltpu.VMEM((2, _FC, D), _BF16),
            pltpu.SemaphoreType.DMA((1,)),
            pltpu.SemaphoreType.DMA((3, 2)),
            pltpu.SemaphoreType.DMA((2,)),
            pltpu.SemaphoreType.DMA((1,)),
        ],
        compiler_params=pltpu.CompilerParams(vmem_limit_bytes=110 * 2**20),
        name="rmt_glu",
    )(
        A_x.reshape(S, D),
        A_mem0.reshape(M, D),
        A_Wq.reshape(D * H, Dh),
        A_Wk.reshape(D * H, Dh),
        A_Wv.reshape(D * H, Dh),
        A_Wo.reshape(H * Dh, D),
        B_w_gate, B_w_up, B_w_down,
    )
    return out.reshape(B, S, D)
```

```python
import functools

import jax
import jax.numpy as jnp
from jax import lax
import jax.experimental.pallas as pl
import jax.experimental.pallas.tpu as pltpu

_F32 = jnp.float32
_BF16 = jnp.bfloat16
_U32 = jnp.uint32

_TB = 256
_FC = 512
_NH = 2
_HG = 4


def _dot(a, b):
    return jnp.dot(a, b, preferred_element_type=_F32)


def _unpack_w(w32):
    return pltpu.bitcast(w32, _BF16)


def _kernel(x_hbm, mem0_ref, wq_hbm, wk_hbm, wv_hbm, wo_hbm, wg_hbm, wu_hbm, wd_hbm,
            out_hbm,
            x_v, xn32, xn16, acc, out_v, wqkv, wo_p, wg_b, wu_b, wd_b, kv_e,
            sem_x, sem_g, sem_w, sem_o,
            *, S, D, H, Dh, M, seg, F):
    n_seg = S // seg
    n_tb = S // _TB
    n_fc = F // _FC
    scale = Dh ** -0.5

    def x_copy(tb):
        rows = pl.ds(tb * _TB, _TB)
        return pltpu.make_async_copy(x_hbm.at[rows, :], x_v.at[rows, :], sem_x.at[tb])

    def glu_copies(fc, slot):
        cols = pl.ds(fc * _FC, _FC)
        return (
            pltpu.make_async_copy(wg_hbm.bitcast(_U32).at[:, cols], wg_b.at[slot], sem_g.at[0, slot]),
            pltpu.make_async_copy(wu_hbm.bitcast(_U32).at[:, cols], wu_b.at[slot], sem_g.at[1, slot]),
            pltpu.make_async_copy(wd_hbm.bitcast(_U32).at[pl.ds(fc * (_FC // 2), _FC // 2), :],
                                  wd_b.at[slot], sem_g.at[2, slot]),
        )

    x_copy(0).start()
    for c in glu_copies(0, 0):
        c.start()
    for tb in range(1, n_tb):
        x_copy(tb).start()
    for c in glu_copies(1, 1):
        c.start()
    for m, w_hbm in enumerate((wq_hbm, wk_hbm, wv_hbm)):
        w32 = w_hbm.bitcast(_U32)
        for j in range(H // 2):
            for par in range(2):
                pltpu.make_async_copy(w32.at[:, par * (H // 2) + j, :], wqkv.at[m, 2 * j + par],
                                      sem_w.at[m]).start()
    wo_cp = pltpu.make_async_copy(wo_hbm.bitcast(_U32), wo_p, sem_w.at[3])
    wo_cp.start()

    def layernorm(tb):
        rows = pl.ds(pl.multiple_of(tb * _TB, _TB), _TB)
        xf = x_v[rows, :].astype(_F32)
        mu = jnp.mean(xf, axis=-1, keepdims=True)
        xc = xf - mu
        var = jnp.mean(xc * xc, axis=-1, keepdims=True)
        xb = (xc * lax.rsqrt(var + 1e-5)).astype(_BF16)
        xn16[rows, :] = xb
        xn32[rows, :] = xb.astype(_F32)

    def glu_unit(tb, slot, first):
        hb = _TB // _NH
        wg = _unpack_w(wg_b[slot])
        wu = _unpack_w(wu_b[slot])
        wd = _unpack_w(wd_b[slot])
        hs = {}
        for a in range(_NH + 1):
            if a < _NH:
                rows = pl.ds(pl.multiple_of(tb * _TB + a * hb, hb), hb)
                xb = xn16[rows, :]
                hs[a] = (jax.nn.sigmoid(_dot(xb, wg)) * _dot(xb, wu)).astype(_BF16)
            if a > 0:
                rows = pl.ds(pl.multiple_of(tb * _TB + (a - 1) * hb, hb), hb)
                y = _dot(hs[a - 1], wd)
                acc[rows, :] = y if first else acc[rows, :] + y

    x_copy(0).wait()
    layernorm(0)
    for c in glu_copies(0, 0):
        c.wait()

    def first_body(tb, carry):
        @pl.when(tb + 1 < n_tb)
        def _():
            x_copy(tb + 1).wait()
        glu_unit(tb, 0, True)
        layernorm(jnp.minimum(tb + 1, n_tb - 1))
        return carry

    lax.fori_loop(0, n_tb, first_body, 0)

    def fc_body(fc, carry):
        slot = fc % 2
        for c in glu_copies(fc, slot):
            c.wait()

        @pl.when(fc + 1 < n_fc)
        def _():
            for c in glu_copies(fc + 1, 1 - slot):
                c.start()

        def tb_body(tb, c2):
            glu_unit(tb, slot, False)
            return c2
        lax.fori_loop(0, n_tb, tb_body, 0)
        return carry

    lax.fori_loop(1, n_fc, fc_body, 0)

    for m in range(3):
        pltpu.make_async_copy(wqkv.at[m], wqkv.at[m], sem_w.at[m]).wait()
    wo_cp.wait()

    def swap_body(u, carry):
        m = u // (H // 2)
        j = u % (H // 2)
        a = wqkv[m, 2 * j]
        b = wqkv[m, 2 * j + 1]
        wqkv[m, 2 * j] = (a & jnp.uint32(0xFFFF)) | (b << 16)
        wqkv[m, 2 * j + 1] = (a >> 16) | (b & jnp.uint32(0xFFFF0000))
        return carry

    lax.fori_loop(0, 3 * (H // 2), swap_body, 0)

    nA = seg - M
    nB = seg + M
    rE = lax.broadcasted_iota(jnp.int32, (seg, M + nB), 0)
    cE = lax.broadcasted_iota(jnp.int32, (seg, M + nB), 1)
    mask_e = ((rE < M) & (cE < M + seg)) | ((rE >= M) & (cE <= rE))
    rO = lax.broadcasted_iota(jnp.int32, (M + nB, 2 * M + 2 * seg), 0)
    cO = lax.broadcasted_iota(jnp.int32, (M + nB, 2 * M + 2 * seg), 1)
    mem2 = (cO >= M + nB) & (cO < 2 * M + nB)
    mask_o = (((rO < M) & (cO >= M + seg))
              | ((rO >= M) & (rO < 2 * M) & (cO <= rO + nA))
              | ((rO >= 2 * M) & (cO >= M + seg)
                 & ((cO <= rO + nA) | mem2 | ((cO >= 2 * M + nB) & (cO <= rO + seg)))))

    def half_step(hq, hk, even):
        G = _HG
        n_g = H // G
        mask = mask_e if even else mask_o
        qkv, probs, outs = {}, {}, {}
        o_acc = None
        for i in range(n_g + 3):
            if i < n_g:
                grp = []
                for h in range(i * G, (i + 1) * G):
                    q = _dot(hq, _unpack_w(wqkv[0, h])).astype(_BF16)
                    k = _dot(hk, _unpack_w(wqkv[1, h])).astype(_BF16)
                    v = _dot(hk, _unpack_w(wqkv[2, h])).astype(_BF16)
                    if even:
                        kv_e[h, 0] = k
                        kv_e[h, 1] = v
                    else:
                        k = jnp.concatenate([kv_e[h, 0], k], axis=0)
                        v = jnp.concatenate([kv_e[h, 1], v], axis=0)
                    grp.append((q, k, v))
                qkv[i] = grp
            g1 = i - 1
            if 0 <= g1 < n_g:
                ps = []
                for (q, k, v) in qkv[g1]:
                    sc = lax.dot_general(q, k, (((1,), (1,)), ((), ())),
                                         preferred_element_type=_F32) * scale
                    sc = jnp.where(mask, sc, -1e9)
                    mx = jnp.max(sc, axis=-1, keepdims=True)
                    e = jnp.exp(sc - mx)
                    ps.append((e / jnp.sum(e, axis=-1, keepdims=True)).astype(_BF16))
                probs[g1] = ps
            g2 = i - 2
            if 0 <= g2 < n_g:
                outs[g2] = jnp.concatenate(
                    [_dot(p, v).astype(_BF16) for p, (_, _, v) in zip(probs[g2], qkv[g2])], axis=1)
            g3 = i - 3
            if 0 <= g3 < n_g:
                r = G * Dh // 2
                y = _dot(outs[g3], _unpack_w(wo_p[g3 * r:(g3 + 1) * r, :]))
                o_acc = y if o_acc is None else o_acc + y
        return o_acc

    def pair_body(j, mem):
        r0 = pl.multiple_of(j * 2 * seg, 2 * seg)
        hk = jnp.concatenate([mem, xn32[pl.ds(r0, nB), :]], axis=0).astype(_BF16)
        ye = half_step(hk[:seg], hk, True)
        mem = ye[:M].astype(_BF16).astype(_F32)
        hq = jnp.concatenate([mem, xn32[pl.ds(r0 + nA, nB), :]], axis=0).astype(_BF16)
        hk = jnp.concatenate([mem, xn32[pl.ds(r0 + nB, nA), :]], axis=0).astype(_BF16)
        yo = half_step(hq, hk, False)
        rows = pl.ds(r0, 2 * seg)
        s_out = jnp.concatenate([ye[M:], yo[M:]], axis=0)
        g = acc[rows, :]
        g = g * jax.nn.sigmoid(g)
        out_v[rows, :] = (x_v[rows, :].astype(_F32) + s_out * g).astype(out_v.dtype)
        pltpu.make_async_copy(out_v.at[rows, :], out_hbm.at[rows, :], sem_o.at[0]).start()
        return yo[:M].astype(_BF16).astype(_F32)

    lax.fori_loop(0, n_seg // 2, pair_body, mem0_ref[...].astype(_F32))
    pltpu.make_async_copy(out_v, out_hbm, sem_o.at[0]).wait()


@functools.partial(jax.jit, static_argnames=("A_seg_len",))
def pallas_recurrent_scan__memory_aug_recurrent_mem_tr__glu_gated_glu__prompt_kernel(
    A_x, A_mem0, A_Wq, A_Wk, A_Wv, A_Wo, A_seg_len, B_x, B_w_gate, B_w_up, B_w_down,
):
    del B_x
    B, S, D = A_x.shape
    _, H, Dh = A_Wq.shape
    M = A_mem0.shape[1]
    F = B_w_gate.shape[1]
    seg = int(A_seg_len)
    assert B == 1 and Dh == 128 and M == 8 and seg == 32 and D == 1024 and H == 32
    assert S % _TB == 0 and F % _FC == 0

    hbm = pl.BlockSpec(memory_space=pl.ANY)
    kern = functools.partial(_kernel, S=S, D=D, H=H, Dh=Dh, M=M, seg=seg, F=F)
    out = pl.pallas_call(
        kern,
        out_shape=jax.ShapeDtypeStruct((S, D), A_x.dtype),
        in_specs=[hbm, pl.BlockSpec(memory_space=pltpu.VMEM), hbm, hbm, hbm, hbm, hbm, hbm, hbm],
        out_specs=hbm,
        scratch_shapes=[
            pltpu.VMEM((S, D), _BF16),
            pltpu.VMEM((S, D), _F32),
            pltpu.VMEM((S, D), _BF16),
            pltpu.VMEM((S, D), _F32),
            pltpu.VMEM((S, D), A_x.dtype),
            pltpu.VMEM((3, H, D // 2, Dh), _U32),
            pltpu.VMEM((H * Dh // 2, D), _U32),
            pltpu.VMEM((2, D // 2, _FC), _U32),
            pltpu.VMEM((2, D // 2, _FC), _U32),
            pltpu.VMEM((2, _FC // 2, D), _U32),
            pltpu.VMEM((H, 2, 2 * M + seg, Dh), _BF16),
            pltpu.SemaphoreType.DMA((S // _TB,)),
            pltpu.SemaphoreType.DMA((3, 2)),
            pltpu.SemaphoreType.DMA((4,)),
            pltpu.SemaphoreType.DMA((1,)),
        ],
        compiler_params=pltpu.CompilerParams(vmem_limit_bytes=110 * 2**20),
        name="rmt_glu",
    )(
        A_x.reshape(S, D),
        A_mem0.reshape(M, D),
        A_Wq.reshape(D // 2, 2 * H, Dh),
        A_Wk.reshape(D // 2, 2 * H, Dh),
        A_Wv.reshape(D // 2, 2 * H, Dh),
        A_Wo.reshape(H * Dh, D),
        B_w_gate, B_w_up, B_w_down,
    )
    return out.reshape(B, S, D)
```

```python
import functools

import jax
import jax.numpy as jnp
from jax import lax
import jax.experimental.pallas as pl
import jax.experimental.pallas.tpu as pltpu

_F32 = jnp.float32
_BF16 = jnp.bfloat16
_U32 = jnp.uint32

_TB = 256
_FC = 512
_NH = 2
_HG = 4


def _dot(a, b):
    return jnp.dot(a, b, preferred_element_type=_F32)


def _unpack_w(w32):
    return pltpu.bitcast(w32, _BF16)


def _kernel(x_hbm, mem0_ref, wq_hbm, wk_hbm, wv_hbm, wo_hbm, wg_hbm, wu_hbm, wd_hbm,
            out_hbm,
            x_v, xn32, xn16, acc, out_v, wqkv, wo_p, wg_b, wu_b, wd_b, kv_e,
            sem_x, sem_g, sem_w, sem_o,
            *, S, D, H, Dh, M, seg, F):
    n_seg = S // seg
    n_tb = S // _TB
    n_fc = F // _FC
    scale = Dh ** -0.5

    def x_copy(tb):
        rows = pl.ds(tb * _TB, _TB)
        return pltpu.make_async_copy(x_hbm.at[rows, :], x_v.at[rows, :], sem_x.at[tb])

    def glu_copies(fc, slot):
        cols = pl.ds(fc * _FC, _FC)
        return (
            pltpu.make_async_copy(wg_hbm.bitcast(_U32).at[:, cols], wg_b.at[slot], sem_g.at[0, slot]),
            pltpu.make_async_copy(wu_hbm.bitcast(_U32).at[:, cols], wu_b.at[slot], sem_g.at[1, slot]),
            pltpu.make_async_copy(wd_hbm.bitcast(_U32).at[pl.ds(fc * (_FC // 2), _FC // 2), :],
                                  wd_b.at[slot], sem_g.at[2, slot]),
        )

    def start_gather(m, w_hbm):
        w32 = w_hbm.bitcast(_U32)

        def body(j, carry):
            for par in range(2):
                pltpu.make_async_copy(w32.at[:, par * (H // 2) + j, :], wqkv.at[m, 2 * j + par],
                                      sem_w.at[m]).start()
            return carry
        lax.fori_loop(0, H // 2, body, 0)

    wo_cp = pltpu.make_async_copy(wo_hbm.bitcast(_U32), wo_p, sem_w.at[3])

    x_copy(0).start()
    for c in glu_copies(0, 0):
        c.start()
    for tb in range(1, n_tb):
        x_copy(tb).start()

    def layernorm(tb):
        rows = pl.ds(pl.multiple_of(tb * _TB, _TB), _TB)
        xf = x_v[rows, :].astype(_F32)
        mu = jnp.mean(xf, axis=-1, keepdims=True)
        xc = xf - mu
        var = jnp.mean(xc * xc, axis=-1, keepdims=True)
        xb = (xc * lax.rsqrt(var + 1e-5)).astype(_BF16)
        xn16[rows, :] = xb
        xn32[rows, :] = xb.astype(_F32)

    def glu_unit(tb, slot, first):
        hb = _TB // _NH
        wg = _unpack_w(wg_b[slot])
        wu = _unpack_w(wu_b[slot])
        wd = _unpack_w(wd_b[slot])
        hs = {}
        for a in range(_NH + 1):
            if a < _NH:
                rows = pl.ds(pl.multiple_of(tb * _TB + a * hb, hb), hb)
                xb = xn16[rows, :]
                hs[a] = (jax.nn.sigmoid(_dot(xb, wg)) * _dot(xb, wu)).astype(_BF16)
            if a > 0:
                rows = pl.ds(pl.multiple_of(tb * _TB + (a - 1) * hb, hb), hb)
                y = _dot(hs[a - 1], wd)
                acc[rows, :] = y if first else acc[rows, :] + y

    x_copy(0).wait()
    layernorm(0)
    for c in glu_copies(0, 0):
        c.wait()

    for c in glu_copies(1, 1):
        c.start()

    def first_body(tb, carry):
        @pl.when(tb + 1 < n_tb)
        def _():
            x_copy(tb + 1).wait()
        glu_unit(tb, 0, True)
        layernorm(jnp.minimum(tb + 1, n_tb - 1))
        return carry

    lax.fori_loop(0, n_tb, first_body, 0)

    def swap_unit(u):
        m = u // (H // 2)
        j = u % (H // 2)
        a = wqkv[m, 2 * j]
        b = wqkv[m, 2 * j + 1]
        wqkv[m, 2 * j] = (a & jnp.uint32(0xFFFF)) | (b << 16)
        wqkv[m, 2 * j + 1] = (a >> 16) | (b & jnp.uint32(0xFFFF0000))

    n_sw_fc = 2
    n_sw = 3 * (H // 2)
    sw_per = -(-n_sw // (n_sw_fc * n_tb))

    def fc_body(fc, carry, *, swap):
        slot = fc % 2
        for c in glu_copies(fc, slot):
            c.wait()

        @pl.when(fc + 1 < n_fc)
        def _():
            for c in glu_copies(fc + 1, 1 - slot):
                c.start()
        if not swap:
            for m, w_hbm in enumerate((wq_hbm, wk_hbm, wv_hbm)):
                pl.when(fc == 1 + m)(functools.partial(start_gather, m, w_hbm))
            pl.when(fc == 4)(wo_cp.start)

        def tb_body(tb, c2):
            glu_unit(tb, slot, False)
            if swap:
                it = (fc - (n_fc - n_sw_fc)) * n_tb + tb
                for r in range(sw_per):
                    swap_unit(it * sw_per + r)
            return c2
        lax.fori_loop(0, n_tb, tb_body, 0)
        return carry

    assert n_fc - n_sw_fc >= 5 and sw_per * n_sw_fc * n_tb == n_sw
    lax.fori_loop(1, n_fc - n_sw_fc, functools.partial(fc_body, swap=False), 0)
    for m in range(3):
        pltpu.make_async_copy(wqkv.at[m], wqkv.at[m], sem_w.at[m]).wait()
    lax.fori_loop(n_fc - n_sw_fc, n_fc, functools.partial(fc_body, swap=True), 0)
    wo_cp.wait()

    nA = seg - M
    nB = seg + M
    rE = lax.broadcasted_iota(jnp.int32, (seg, M + nB), 0)
    cE = lax.broadcasted_iota(jnp.int32, (seg, M + nB), 1)
    mask_e = ((rE < M) & (cE < M + seg)) | ((rE >= M) & (cE <= rE))
    rO = lax.broadcasted_iota(jnp.int32, (M + nB, 2 * M + 2 * seg), 0)
    cO = lax.broadcasted_iota(jnp.int32, (M + nB, 2 * M + 2 * seg), 1)
    mem2 = (cO >= M + nB) & (cO < 2 * M + nB)
    mask_o = (((rO < M) & (cO >= M + seg))
              | ((rO >= M) & (rO < 2 * M) & (cO <= rO + nA))
              | ((rO >= 2 * M) & (cO >= M + seg)
                 & ((cO <= rO + nA) | mem2 | ((cO >= 2 * M + nB) & (cO <= rO + seg)))))

    def half_step(hq, hk, even):
        G = _HG
        n_g = H // G
        mask = mask_e if even else mask_o
        qkv, probs, outs = {}, {}, {}
        o_acc = None
        for i in range(n_g + 3):
            if i < n_g:
                grp = []
                for h in range(i * G, (i + 1) * G):
                    q = _dot(hq, _unpack_w(wqkv[0, h])).astype(_BF16)
                    k = _dot(hk, _unpack_w(wqkv[1, h])).astype(_BF16)
                    v = _dot(hk, _unpack_w(wqkv[2, h])).astype(_BF16)
                    if even:
                        kv_e[h, 0] = k
                        kv_e[h, 1] = v
                    else:
                        k = jnp.concatenate([kv_e[h, 0], k], axis=0)
                        v = jnp.concatenate([kv_e[h, 1], v], axis=0)
                    grp.append((q, k, v))
                qkv[i] = grp
            g1 = i - 1
            if 0 <= g1 < n_g:
                ps = []
                for (q, k, v) in qkv[g1]:
                    sc = lax.dot_general(q, k, (((1,), (1,)), ((), ())),
                                         preferred_element_type=_F32) * scale
                    sc = jnp.where(mask, sc, -1e9)
                    mx = jnp.max(sc, axis=-1, keepdims=True)
                    e = jnp.exp(sc - mx)
                    ps.append((e / jnp.sum(e, axis=-1, keepdims=True)).astype(_BF16))
                probs[g1] = ps
            g2 = i - 2
            if 0 <= g2 < n_g:
                outs[g2] = jnp.concatenate(
                    [_dot(p, v).astype(_BF16) for p, (_, _, v) in zip(probs[g2], qkv[g2])], axis=1)
            g3 = i - 3
            if 0 <= g3 < n_g:
                r = G * Dh // 2
                y = _dot(outs[g3], _unpack_w(wo_p[g3 * r:(g3 + 1) * r, :]))
                o_acc = y if o_acc is None else o_acc + y
        return o_acc

    def pair_body(j, mem):
        r0 = pl.multiple_of(j * 2 * seg, 2 * seg)
        hk = jnp.concatenate([mem, xn32[pl.ds(r0, nB), :]], axis=0).astype(_BF16)
        ye = half_step(hk[:seg], hk, True)
        mem = ye[:M].astype(_BF16).astype(_F32)
        hq = jnp.concatenate([mem, xn32[pl.ds(r0 + nA, nB), :]], axis=0).astype(_BF16)
        hk = jnp.concatenate([mem, xn32[pl.ds(r0 + nB, nA), :]], axis=0).astype(_BF16)
        yo = half_step(hq, hk, False)
        rows = pl.ds(r0, 2 * seg)
        s_out = jnp.concatenate([ye[M:], yo[M:]], axis=0)
        g = acc[rows, :]
        g = g * jax.nn.sigmoid(g)
        out_v[rows, :] = (x_v[rows, :].astype(_F32) + s_out * g).astype(out_v.dtype)
        pltpu.make_async_copy(out_v.at[rows, :], out_hbm.at[rows, :], sem_o.at[0]).start()
        return yo[:M].astype(_BF16).astype(_F32)

    lax.fori_loop(0, n_seg // 2, pair_body, mem0_ref[...].astype(_F32))
    pltpu.make_async_copy(out_v, out_hbm, sem_o.at[0]).wait()


@functools.partial(jax.jit, static_argnames=("A_seg_len",))
def pallas_recurrent_scan__memory_aug_recurrent_mem_tr__glu_gated_glu__prompt_kernel(
    A_x, A_mem0, A_Wq, A_Wk, A_Wv, A_Wo, A_seg_len, B_x, B_w_gate, B_w_up, B_w_down,
):
    del B_x
    B, S, D = A_x.shape
    _, H, Dh = A_Wq.shape
    M = A_mem0.shape[1]
    F = B_w_gate.shape[1]
    seg = int(A_seg_len)
    assert B == 1 and Dh == 128 and M == 8 and seg == 32 and D == 1024 and H == 32
    assert S % _TB == 0 and F % _FC == 0

    hbm = pl.BlockSpec(memory_space=pl.ANY)
    kern = functools.partial(_kernel, S=S, D=D, H=H, Dh=Dh, M=M, seg=seg, F=F)
    out = pl.pallas_call(
        kern,
        out_shape=jax.ShapeDtypeStruct((S, D), A_x.dtype),
        in_specs=[hbm, pl.BlockSpec(memory_space=pltpu.VMEM), hbm, hbm, hbm, hbm, hbm, hbm, hbm],
        out_specs=hbm,
        scratch_shapes=[
            pltpu.VMEM((S, D), _BF16),
            pltpu.VMEM((S, D), _F32),
            pltpu.VMEM((S, D), _BF16),
            pltpu.VMEM((S, D), _F32),
            pltpu.VMEM((S, D), A_x.dtype),
            pltpu.VMEM((3, H, D // 2, Dh), _U32),
            pltpu.VMEM((H * Dh // 2, D), _U32),
            pltpu.VMEM((2, D // 2, _FC), _U32),
            pltpu.VMEM((2, D // 2, _FC), _U32),
            pltpu.VMEM((2, _FC // 2, D), _U32),
            pltpu.VMEM((H, 2, 2 * M + seg, Dh), _BF16),
            pltpu.SemaphoreType.DMA((S // _TB,)),
            pltpu.SemaphoreType.DMA((3, 2)),
            pltpu.SemaphoreType.DMA((4,)),
            pltpu.SemaphoreType.DMA((1,)),
        ],
        compiler_params=pltpu.CompilerParams(vmem_limit_bytes=110 * 2**20),
        name="rmt_glu",
    )(
        A_x.reshape(S, D),
        A_mem0.reshape(M, D),
        A_Wq.reshape(D // 2, 2 * H, Dh),
        A_Wk.reshape(D // 2, 2 * H, Dh),
        A_Wv.reshape(D // 2, 2 * H, Dh),
        A_Wo.reshape(H * Dh, D),
        B_w_gate, B_w_up, B_w_down,
    )
    return out.reshape(B, S, D)
```

```python
import functools

import jax
import jax.numpy as jnp
from jax import lax
import jax.experimental.pallas as pl
import jax.experimental.pallas.tpu as pltpu

_F32 = jnp.float32
_BF16 = jnp.bfloat16
_U32 = jnp.uint32

_TB = 512
_FC = 512
_NH = 4
_HG = 4


def _dot(a, b):
    return jnp.dot(a, b, preferred_element_type=_F32)


def _unpack_w(w32):
    return pltpu.bitcast(w32, _BF16)


def _kernel(x_hbm, mem0_ref, wq_hbm, wk_hbm, wv_hbm, wo_hbm, wg_hbm, wu_hbm, wd_hbm,
            out_hbm,
            x_v, xn32, xn16, acc, out_v, wqkv, wo_p, wg_b, wu_b, wd_b, kv_e, h_last, s_buf,
            sem_x, sem_g, sem_w, sem_o,
            *, S, D, H, Dh, M, seg, F):
    n_seg = S // seg
    n_tb = S // _TB
    n_fc = F // _FC
    scale = Dh ** -0.5

    def x_copy(tb):
        rows = pl.ds(tb * _TB, _TB)
        return pltpu.make_async_copy(x_hbm.at[rows, :], x_v.at[rows, :], sem_x.at[tb])

    def glu_copies(fc, slot):
        cols = pl.ds(fc * _FC, _FC)
        return (
            pltpu.make_async_copy(wg_hbm.bitcast(_U32).at[:, cols], wg_b.at[slot], sem_g.at[0, slot]),
            pltpu.make_async_copy(wu_hbm.bitcast(_U32).at[:, cols], wu_b.at[slot], sem_g.at[1, slot]),
            pltpu.make_async_copy(wd_hbm.bitcast(_U32).at[pl.ds(fc * (_FC // 2), _FC // 2), :],
                                  wd_b.at[slot], sem_g.at[2, slot]),
        )

    def start_gather(m, w_hbm):
        w32 = w_hbm.bitcast(_U32)

        def body(j, carry):
            for par in range(2):
                pltpu.make_async_copy(w32.at[:, par * (H // 2) + j, :], wqkv.at[m, 2 * j + par],
                                      sem_w.at[m]).start()
            return carry
        lax.fori_loop(0, H // 2, body, 0)

    wo_cp = pltpu.make_async_copy(wo_hbm.bitcast(_U32), wo_p, sem_w.at[3])

    x_copy(0).start()
    for c in glu_copies(0, 0):
        c.start()
    for tb in range(1, n_tb):
        x_copy(tb).start()

    def layernorm(tb):
        rows = pl.ds(pl.multiple_of(tb * _TB, _TB), _TB)
        xf = x_v[rows, :].astype(_F32)
        mu = jnp.mean(xf, axis=-1, keepdims=True)
        xc = xf - mu
        var = jnp.mean(xc * xc, axis=-1, keepdims=True)
        xb = (xc * lax.rsqrt(var + 1e-5)).astype(_BF16)
        xn16[rows, :] = xb
        xn32[rows, :] = xb.astype(_F32)

    def glu_unit(tb, slot, first, defer=False, extra=()):
        hb = _TB // _NH
        wg = _unpack_w(wg_b[slot])
        wu = _unpack_w(wu_b[slot])
        wd = _unpack_w(wd_b[slot])
        hs = {}
        for a in range(_NH + 1):
            if a < _NH:
                rows = pl.ds(pl.multiple_of(tb * _TB + a * hb, hb), hb)
                xb = xn16[rows, :]
                hs[a] = (jax.nn.sigmoid(_dot(xb, wg)) * _dot(xb, wu)).astype(_BF16)
                if a < len(extra):
                    extra[a]()
            if a > 0:
                rows = pl.ds(pl.multiple_of(tb * _TB + (a - 1) * hb, hb), hb)
                if defer:
                    h_last[rows, :] = hs[a - 1]
                    continue
                y = _dot(hs[a - 1], wd)
                acc[rows, :] = y if first else acc[rows, :] + y

    x_copy(0).wait()
    layernorm(0)
    for c in glu_copies(0, 0):
        c.wait()

    for c in glu_copies(1, 1):
        c.start()

    def first_body(tb, carry):
        @pl.when(tb + 1 < n_tb)
        def _():
            x_copy(tb + 1).wait()
        glu_unit(tb, 0, True)
        layernorm(jnp.minimum(tb + 1, n_tb - 1))
        return carry

    lax.fori_loop(0, n_tb, first_body, 0)

    def swap_unit(u):
        m = u // (H // 2)
        j = u % (H // 2)
        a = wqkv[m, 2 * j]
        b = wqkv[m, 2 * j + 1]
        wqkv[m, 2 * j] = (a & jnp.uint32(0xFFFF)) | (b << 16)
        wqkv[m, 2 * j + 1] = (a >> 16) | (b & jnp.uint32(0xFFFF0000))

    n_sw = 3 * (H // 2)
    sw_per = n_sw // (2 * n_tb)

    def fc_body(fc, carry, *, swap, defer=False):
        slot = fc % 2
        for c in glu_copies(fc, slot):
            c.wait()

        if not defer:
            for c in glu_copies(fc + 1, 1 - slot):
                c.start()
        if not swap:
            for m, w_hbm in enumerate((wq_hbm, wk_hbm, wv_hbm)):
                pl.when(fc == 1 + m)(functools.partial(start_gather, m, w_hbm))
            pl.when(fc == 4)(wo_cp.start)

        def tb_body(tb, c2):
            extra = []
            if swap:
                it = (fc - (n_fc - 2)) * n_tb + tb
                per = -(-sw_per // _NH)

                def mk(a):
                    def go():
                        for r in range(min(per, sw_per - a * per)):
                            swap_unit(it * sw_per + a * per + r)
                    return go
                extra = [mk(a) for a in range(_NH)]
            glu_unit(tb, slot, False, defer, extra)
            return c2
        lax.fori_loop(0, n_tb, tb_body, 0)
        return carry

    assert n_fc >= 7 and sw_per * 2 * n_tb == n_sw
    lax.fori_loop(1, n_fc - 2, functools.partial(fc_body, swap=False), 0)
    for m in range(3):
        pltpu.make_async_copy(wqkv.at[m], wqkv.at[m], sem_w.at[m]).wait()
    fc_body(n_fc - 2, 0, swap=True)
    fc_body(n_fc - 1, 0, swap=True, defer=True)
    wo_cp.wait()
    last_slot = (n_fc - 1) % 2

    nA = seg - M
    nB = seg + M
    rE = lax.broadcasted_iota(jnp.int32, (seg, M + nB), 0)
    cE = lax.broadcasted_iota(jnp.int32, (seg, M + nB), 1)
    mask_e = ((rE < M) & (cE < M + seg)) | ((rE >= M) & (cE <= rE))
    rO = lax.broadcasted_iota(jnp.int32, (M + nB, 2 * M + 2 * seg), 0)
    cO = lax.broadcasted_iota(jnp.int32, (M + nB, 2 * M + 2 * seg), 1)
    mem2 = (cO >= M + nB) & (cO < 2 * M + nB)
    mask_o = (((rO < M) & (cO >= M + seg))
              | ((rO >= M) & (rO < 2 * M) & (cO <= rO + nA))
              | ((rO >= 2 * M) & (cO >= M + seg)
                 & ((cO <= rO + nA) | mem2 | ((cO >= 2 * M + nB) & (cO <= rO + seg)))))

    def half_step(hq, hk, even, fill=None):
        G = _HG
        n_g = H // G
        mask = mask_e if even else mask_o
        qkv, probs, outs = {}, {}, {}
        o_acc = None
        fill = fill or {}
        for i in range(n_g + 3):
            if i < n_g:
                grp = []
                for h in range(i * G, (i + 1) * G):
                    q = _dot(hq, _unpack_w(wqkv[0, h])).astype(_BF16)
                    k = _dot(hk, _unpack_w(wqkv[1, h])).astype(_BF16)
                    v = _dot(hk, _unpack_w(wqkv[2, h])).astype(_BF16)
                    if even:
                        kv_e[h, 0] = k
                        kv_e[h, 1] = v
                    else:
                        k = jnp.concatenate([kv_e[h, 0], k], axis=0)
                        v = jnp.concatenate([kv_e[h, 1], v], axis=0)
                    grp.append((q, k, v))
                qkv[i] = grp
            g1 = i - 1
            if 0 <= g1 < n_g:
                ps = []
                for (q, k, v) in qkv[g1]:
                    sc = lax.dot_general(q, k, (((1,), (1,)), ((), ())),
                                         preferred_element_type=_F32) * scale
                    sc = jnp.where(mask, sc, -1e9)
                    mx = jnp.max(sc, axis=-1, keepdims=True)
                    e = jnp.exp(sc - mx)
                    ps.append((e.astype(_BF16), 1.0 / jnp.sum(e, axis=-1, keepdims=True)))
                probs[g1] = ps
            if (i, 0) in fill:
                fill[(i, 0)]()
            g2 = i - 2
            if 0 <= g2 < n_g:
                outs[g2] = jnp.concatenate(
                    [(_dot(p, v) * inv).astype(_BF16) for (p, inv), (_, _, v) in zip(probs[g2], qkv[g2])], axis=1)
            if (i, 1) in fill:
                fill[(i, 1)]()
            g3 = i - 3
            if 0 <= g3 < n_g:
                r = G * Dh // 2
                y = _dot(outs[g3], _unpack_w(wo_p[g3 * r:(g3 + 1) * r, :]))
                o_acc = y if o_acc is None else o_acc + y
        return o_acc

    def glu_tail(r0, c0=0, nc=D):
        rows = pl.ds(pl.multiple_of(r0, seg), seg)
        cols = slice(c0, c0 + nc)
        acc[rows, cols] += _dot(h_last[rows, :], _unpack_w(wd_b[last_slot, :, cols]))

    def epilogue(j):
        rows = pl.ds(pl.multiple_of(j * 2 * seg, 2 * seg), 2 * seg)
        g = acc[rows, :]
        g = g * jax.nn.sigmoid(g)
        out_v[rows, :] = (x_v[rows, :].astype(_F32) + s_buf[...] * g).astype(out_v.dtype)

    def out_copy(j):
        rows = pl.ds(pl.multiple_of(j * 2 * seg, 2 * seg), 2 * seg)
        return pltpu.make_async_copy(out_v.at[rows, :], out_hbm.at[rows, :], sem_o.at[0])

    def pair_body(j, mem):
        r0 = pl.multiple_of(j * 2 * seg, 2 * seg)
        hk = jnp.concatenate([mem, xn32[pl.ds(r0, nB), :]], axis=0).astype(_BF16)
        epilogue(jnp.maximum(j - 1, 0))
        n_g = H // _HG
        ye = half_step(hk[:seg], hk, True, {
            (n_g + 1, 0): functools.partial(glu_tail, r0, 0, D // 2),
            (n_g + 2, 1): functools.partial(glu_tail, r0, D // 2, D // 2)})
        glu_tail(r0 + seg)
        mem = ye[:M].astype(_BF16).astype(_F32)
        hq = jnp.concatenate([mem, xn32[pl.ds(r0 + nA, nB), :]], axis=0).astype(_BF16)
        hk = jnp.concatenate([mem, xn32[pl.ds(r0 + nB, nA), :]], axis=0).astype(_BF16)
        yo = half_step(hq, hk, False)
        s_buf[...] = jnp.concatenate([ye[M:], yo[M:]], axis=0)

        @pl.when(j > 0)
        def _():
            out_copy(j - 1).start()
        return yo[:M].astype(_BF16).astype(_F32)

    s_buf[...] = jnp.zeros_like(s_buf)
    lax.fori_loop(0, n_seg // 2, pair_body, mem0_ref[...].astype(_F32))
    epilogue(n_seg // 2 - 1)
    out_copy(n_seg // 2 - 1).start()
    pltpu.make_async_copy(out_v, out_hbm, sem_o.at[0]).wait()


@functools.partial(jax.jit, static_argnames=("A_seg_len",))
def pallas_recurrent_scan__memory_aug_recurrent_mem_tr__glu_gated_glu__prompt_kernel(
    A_x, A_mem0, A_Wq, A_Wk, A_Wv, A_Wo, A_seg_len, B_x, B_w_gate, B_w_up, B_w_down,
):
    del B_x
    B, S, D = A_x.shape
    _, H, Dh = A_Wq.shape
    M = A_mem0.shape[1]
    F = B_w_gate.shape[1]
    seg = int(A_seg_len)
    assert B == 1 and Dh == 128 and M == 8 and seg == 32 and D == 1024 and H == 32
    assert S % _TB == 0 and F % _FC == 0

    hbm = pl.BlockSpec(memory_space=pl.ANY)
    kern = functools.partial(_kernel, S=S, D=D, H=H, Dh=Dh, M=M, seg=seg, F=F)
    out = pl.pallas_call(
        kern,
        out_shape=jax.ShapeDtypeStruct((S, D), A_x.dtype),
        in_specs=[hbm, pl.BlockSpec(memory_space=pltpu.VMEM), hbm, hbm, hbm, hbm, hbm, hbm, hbm],
        out_specs=hbm,
        scratch_shapes=[
            pltpu.VMEM((S, D), _BF16),
            pltpu.VMEM((S, D), _F32),
            pltpu.VMEM((S, D), _BF16),
            pltpu.VMEM((S, D), _F32),
            pltpu.VMEM((S, D), A_x.dtype),
            pltpu.VMEM((3, H, D // 2, Dh), _U32),
            pltpu.VMEM((H * Dh // 2, D), _U32),
            pltpu.VMEM((2, D // 2, _FC), _U32),
            pltpu.VMEM((2, D // 2, _FC), _U32),
            pltpu.VMEM((2, _FC // 2, D), _U32),
            pltpu.VMEM((H, 2, 2 * M + seg, Dh), _BF16),
            pltpu.VMEM((S, _FC), _BF16),
            pltpu.VMEM((2 * seg, D), _F32),
            pltpu.SemaphoreType.DMA((S // _TB,)),
            pltpu.SemaphoreType.DMA((3, 2)),
            pltpu.SemaphoreType.DMA((4,)),
            pltpu.SemaphoreType.DMA((1,)),
        ],
        compiler_params=pltpu.CompilerParams(vmem_limit_bytes=110 * 2**20),
        name="rmt_glu",
    )(
        A_x.reshape(S, D),
        A_mem0.reshape(M, D),
        A_Wq.reshape(D // 2, 2 * H, Dh),
        A_Wk.reshape(D // 2, 2 * H, Dh),
        A_Wv.reshape(D // 2, 2 * H, Dh),
        A_Wo.reshape(H * Dh, D),
        B_w_gate, B_w_up, B_w_down,
    )
    return out.reshape(B, S, D)
```

```python
import functools

import jax
import jax.numpy as jnp
from jax import lax
import jax.experimental.pallas as pl
import jax.experimental.pallas.tpu as pltpu

_F32 = jnp.float32
_BF16 = jnp.bfloat16
_U32 = jnp.uint32

_TB = 512
_FC = 512
_NH = 4
_HG = 4


def _dot(a, b):
    return jnp.dot(a, b, preferred_element_type=_F32)


def _unpack_w(w32):
    return pltpu.bitcast(w32, _BF16)


def _kernel(x_hbm, mem0_ref, wq_hbm, wk_hbm, wv_hbm, wo_hbm, wg_hbm, wu_hbm, wd_hbm,
            out_hbm,
            x_v, xn32, xn16, acc, out_v, wqkv, wo_p, wg_b, wu_b, wd_b, kv_e, h_last, s_buf,
            sem_x, sem_g, sem_w, sem_o,
            *, S, D, H, Dh, M, seg, F):
    n_seg = S // seg
    n_tb = S // _TB
    n_fc = F // _FC
    scale = Dh ** -0.5

    def x_copy(tb):
        rows = pl.ds(tb * _TB, _TB)
        return pltpu.make_async_copy(x_hbm.at[rows, :], x_v.at[rows, :], sem_x.at[tb])

    def glu_copies(fc, slot):
        cols = pl.ds(fc * _FC, _FC)
        return (
            pltpu.make_async_copy(wg_hbm.bitcast(_U32).at[:, cols], wg_b.at[slot], sem_g.at[0, slot]),
            pltpu.make_async_copy(wu_hbm.bitcast(_U32).at[:, cols], wu_b.at[slot], sem_g.at[1, slot]),
            pltpu.make_async_copy(wd_hbm.bitcast(_U32).at[pl.ds(fc * (_FC // 2), _FC // 2), :],
                                  wd_b.at[slot], sem_g.at[2, slot]),
        )

    def start_gather(m, w_hbm):
        w32 = w_hbm.bitcast(_U32)

        def body(j, carry):
            for par in range(2):
                pltpu.make_async_copy(w32.at[:, par * (H // 2) + j, :], wqkv.at[m, 2 * j + par],
                                      sem_w.at[m]).start()
            return carry
        lax.fori_loop(0, H // 2, body, 0)

    wo_cp = pltpu.make_async_copy(wo_hbm.bitcast(_U32), wo_p, sem_w.at[3])

    x_copy(0).start()
    for c in glu_copies(0, 0):
        c.start()
    for tb in range(1, n_tb):
        x_copy(tb).start()

    def layernorm(tb, a=None):
        if a is None:
            rows = pl.ds(pl.multiple_of(tb * _TB, _TB), _TB)
        else:
            hb = _TB // _NH
            rows = pl.ds(pl.multiple_of(tb * _TB + a * hb, hb), hb)
        xf = x_v[rows, :].astype(_F32)
        mu = jnp.mean(xf, axis=-1, keepdims=True)
        xc = xf - mu
        var = jnp.mean(xc * xc, axis=-1, keepdims=True)
        xb = (xc * lax.rsqrt(var + 1e-5)).astype(_BF16)
        xn16[rows, :] = xb
        xn32[rows, :] = xb.astype(_F32)

    def glu_unit(tb, slot, first, defer=False, extra=()):
        hb = _TB // _NH
        wg = _unpack_w(wg_b[slot])
        wu = _unpack_w(wu_b[slot])
        wd = _unpack_w(wd_b[slot])
        hs = {}
        if first:
            xall = xn16[pl.ds(pl.multiple_of(tb * _TB, _TB), _TB), :]
        for a in range(_NH + 1):
            if a < _NH:
                rows = pl.ds(pl.multiple_of(tb * _TB + a * hb, hb), hb)
                xb = xall[a * hb:(a + 1) * hb] if first else xn16[rows, :]
                hs[a] = (jax.nn.sigmoid(_dot(xb, wg)) * _dot(xb, wu)).astype(_BF16)
                if a < len(extra):
                    extra[a]()
            if a > 0:
                rows = pl.ds(pl.multiple_of(tb * _TB + (a - 1) * hb, hb), hb)
                if defer:
                    h_last[rows, :] = hs[a - 1]
                    continue
                y = _dot(hs[a - 1], wd)
                acc[rows, :] = y if first else acc[rows, :] + y

    x_copy(0).wait()
    layernorm(0)
    for c in glu_copies(0, 0):
        c.wait()

    for c in glu_copies(1, 1):
        c.start()

    def first_body(tb, carry):
        @pl.when(tb + 1 < n_tb)
        def _():
            x_copy(tb + 1).wait()
        nxt = jnp.minimum(tb + 1, n_tb - 1)
        glu_unit(tb, 0, True, False, [functools.partial(layernorm, nxt, a) for a in range(_NH)])
        return carry

    lax.fori_loop(0, n_tb, first_body, 0)

    def swap_unit(u):
        m = u // (H // 2)
        j = u % (H // 2)
        a = wqkv[m, 2 * j]
        b = wqkv[m, 2 * j + 1]
        wqkv[m, 2 * j] = (a & jnp.uint32(0xFFFF)) | (b << 16)
        wqkv[m, 2 * j + 1] = (a >> 16) | (b & jnp.uint32(0xFFFF0000))

    n_sw = 3 * (H // 2)
    sw_per = n_sw // (2 * n_tb)

    def fc_body(fc, carry, *, swap, defer=False):
        slot = fc % 2
        for c in glu_copies(fc, slot):
            c.wait()

        if not defer:
            for c in glu_copies(fc + 1, 1 - slot):
                c.start()
        if not swap:
            for m, w_hbm in enumerate((wq_hbm, wk_hbm, wv_hbm)):
                pl.when(fc == 1 + m)(functools.partial(start_gather, m, w_hbm))
            pl.when(fc == 4)(wo_cp.start)

        def tb_body(tb, c2):
            extra = []
            if swap:
                it = (fc - (n_fc - 2)) * n_tb + tb
                per = -(-sw_per // _NH)

                def mk(a):
                    def go():
                        for r in range(min(per, sw_per - a * per)):
                            swap_unit(it * sw_per + a * per + r)
                    return go
                extra = [mk(a) for a in range(_NH)]
            glu_unit(tb, slot, False, defer, extra)
            return c2
        lax.fori_loop(0, n_tb, tb_body, 0)
        return carry

    assert n_fc >= 7 and sw_per * 2 * n_tb == n_sw
    lax.fori_loop(1, n_fc - 2, functools.partial(fc_body, swap=False), 0)
    for m in range(3):
        pltpu.make_async_copy(wqkv.at[m], wqkv.at[m], sem_w.at[m]).wait()
    fc_body(n_fc - 2, 0, swap=True)
    fc_body(n_fc - 1, 0, swap=True, defer=True)
    wo_cp.wait()
    last_slot = (n_fc - 1) % 2

    nA = seg - M
    nB = seg + M
    rE = lax.broadcasted_iota(jnp.int32, (seg, M + nB), 0)
    cE = lax.broadcasted_iota(jnp.int32, (seg, M + nB), 1)
    mask_e = ((rE < M) & (cE < M + seg)) | ((rE >= M) & (cE <= rE))
    rO = lax.broadcasted_iota(jnp.int32, (M + nB, 2 * M + 2 * seg), 0)
    cO = lax.broadcasted_iota(jnp.int32, (M + nB, 2 * M + 2 * seg), 1)
    mem2 = (cO >= M + nB) & (cO < 2 * M + nB)
    mask_o = (((rO < M) & (cO >= M + seg))
              | ((rO >= M) & (rO < 2 * M) & (cO <= rO + nA))
              | ((rO >= 2 * M) & (cO >= M + seg)
                 & ((cO <= rO + nA) | mem2 | ((cO >= 2 * M + nB) & (cO <= rO + seg)))))

    def half_step(hq, hk, even, fill=None):
        G = _HG
        n_g = H // G
        mask = mask_e if even else mask_o
        qkv, probs, outs = {}, {}, {}
        o_acc = None
        fill = fill or {}
        for i in range(n_g + 3):
            if i < n_g:
                grp = []
                for h in range(i * G, (i + 1) * G):
                    q = _dot(hq, _unpack_w(wqkv[0, h])).astype(_BF16)
                    k = _dot(hk, _unpack_w(wqkv[1, h])).astype(_BF16)
                    v = _dot(hk, _unpack_w(wqkv[2, h])).astype(_BF16)
                    if even:
                        kv_e[h, 0] = k
                        kv_e[h, 1] = v
                    else:
                        k = jnp.concatenate([kv_e[h, 0], k], axis=0)
                        v = jnp.concatenate([kv_e[h, 1], v], axis=0)
                    grp.append((q, k, v))
                qkv[i] = grp
            g1 = i - 1
            if 0 <= g1 < n_g:
                ps = []
                for (q, k, v) in qkv[g1]:
                    sc = lax.dot_general(q, k, (((1,), (1,)), ((), ())),
                                         preferred_element_type=_F32) * scale
                    sc = jnp.where(mask, sc, -1e9)
                    mx = jnp.max(sc, axis=-1, keepdims=True)
                    e = jnp.exp(sc - mx)
                    ps.append((e.astype(_BF16), 1.0 / jnp.sum(e, axis=-1, keepdims=True)))
                probs[g1] = ps
            if (i, 0) in fill:
                fill[(i, 0)]()
            g2 = i - 2
            if 0 <= g2 < n_g:
                outs[g2] = jnp.concatenate(
                    [(_dot(p, v) * inv).astype(_BF16) for (p, inv), (_, _, v) in zip(probs[g2], qkv[g2])], axis=1)
            if (i, 1) in fill:
                fill[(i, 1)]()
            g3 = i - 3
            if 0 <= g3 < n_g:
                r = G * Dh // 2
                y = _dot(outs[g3], _unpack_w(wo_p[g3 * r:(g3 + 1) * r, :]))
                o_acc = y if o_acc is None else o_acc + y
        return o_acc

    def glu_tail(r0, c0=0, nc=D):
        rows = pl.ds(pl.multiple_of(r0, seg), seg)
        cols = slice(c0, c0 + nc)
        acc[rows, cols] += _dot(h_last[rows, :], _unpack_w(wd_b[last_slot, :, cols]))

    def epilogue(j):
        rows = pl.ds(pl.multiple_of(j * 2 * seg, 2 * seg), 2 * seg)
        g = acc[rows, :]
        g = g * jax.nn.sigmoid(g)
        out_v[rows, :] = (x_v[rows, :].astype(_F32) + s_buf[...] * g).astype(out_v.dtype)

    def out_copy(j):
        rows = pl.ds(pl.multiple_of(j * 2 * seg, 2 * seg), 2 * seg)
        return pltpu.make_async_copy(out_v.at[rows, :], out_hbm.at[rows, :], sem_o.at[0])

    def pair_body(j, mem):
        r0 = pl.multiple_of(j * 2 * seg, 2 * seg)
        hk = jnp.concatenate([mem, xn32[pl.ds(r0, nB), :]], axis=0).astype(_BF16)
        epilogue(jnp.maximum(j - 1, 0))
        n_g = H // _HG
        ye = half_step(hk[:seg], hk, True, {
            (n_g + 1, 0): functools.partial(glu_tail, r0, 0, D // 2),
            (n_g + 2, 1): functools.partial(glu_tail, r0, D // 2, D // 2)})
        glu_tail(r0 + seg)
        mem = ye[:M].astype(_BF16).astype(_F32)
        hq = jnp.concatenate([mem, xn32[pl.ds(r0 + nA, nB), :]], axis=0).astype(_BF16)
        hk = jnp.concatenate([mem, xn32[pl.ds(r0 + nB, nA), :]], axis=0).astype(_BF16)
        yo = half_step(hq, hk, False)
        s_buf[...] = jnp.concatenate([ye[M:], yo[M:]], axis=0)

        @pl.when(j > 0)
        def _():
            out_copy(j - 1).start()
        return yo[:M].astype(_BF16).astype(_F32)

    s_buf[...] = jnp.zeros_like(s_buf)
    lax.fori_loop(0, n_seg // 2, pair_body, mem0_ref[...].astype(_F32))
    epilogue(n_seg // 2 - 1)
    out_copy(n_seg // 2 - 1).start()
    pltpu.make_async_copy(out_v, out_hbm, sem_o.at[0]).wait()


@functools.partial(jax.jit, static_argnames=("A_seg_len",))
def pallas_recurrent_scan__memory_aug_recurrent_mem_tr__glu_gated_glu__prompt_kernel(
    A_x, A_mem0, A_Wq, A_Wk, A_Wv, A_Wo, A_seg_len, B_x, B_w_gate, B_w_up, B_w_down,
):
    del B_x
    B, S, D = A_x.shape
    _, H, Dh = A_Wq.shape
    M = A_mem0.shape[1]
    F = B_w_gate.shape[1]
    seg = int(A_seg_len)
    assert B == 1 and Dh == 128 and M == 8 and seg == 32 and D == 1024 and H == 32
    assert S % _TB == 0 and F % _FC == 0

    hbm = pl.BlockSpec(memory_space=pl.ANY)
    kern = functools.partial(_kernel, S=S, D=D, H=H, Dh=Dh, M=M, seg=seg, F=F)
    out = pl.pallas_call(
        kern,
        out_shape=jax.ShapeDtypeStruct((S, D), A_x.dtype),
        in_specs=[hbm, pl.BlockSpec(memory_space=pltpu.VMEM), hbm, hbm, hbm, hbm, hbm, hbm, hbm],
        out_specs=hbm,
        scratch_shapes=[
            pltpu.VMEM((S, D), _BF16),
            pltpu.VMEM((S, D), _F32),
            pltpu.VMEM((S, D), _BF16),
            pltpu.VMEM((S, D), _F32),
            pltpu.VMEM((S, D), A_x.dtype),
            pltpu.VMEM((3, H, D // 2, Dh), _U32),
            pltpu.VMEM((H * Dh // 2, D), _U32),
            pltpu.VMEM((2, D // 2, _FC), _U32),
            pltpu.VMEM((2, D // 2, _FC), _U32),
            pltpu.VMEM((2, _FC // 2, D), _U32),
            pltpu.VMEM((H, 2, 2 * M + seg, Dh), _BF16),
            pltpu.VMEM((S, _FC), _BF16),
            pltpu.VMEM((2 * seg, D), _F32),
            pltpu.SemaphoreType.DMA((S // _TB,)),
            pltpu.SemaphoreType.DMA((3, 2)),
            pltpu.SemaphoreType.DMA((4,)),
            pltpu.SemaphoreType.DMA((1,)),
        ],
        compiler_params=pltpu.CompilerParams(vmem_limit_bytes=110 * 2**20),
        name="rmt_glu",
    )(
        A_x.reshape(S, D),
        A_mem0.reshape(M, D),
        A_Wq.reshape(D // 2, 2 * H, Dh),
        A_Wk.reshape(D // 2, 2 * H, Dh),
        A_Wv.reshape(D // 2, 2 * H, Dh),
        A_Wo.reshape(H * Dh, D),
        B_w_gate, B_w_up, B_w_down,
    )
    return out.reshape(B, S, D)
```
